```python
import jax
import jax.numpy as jnp

def _softmax(x, axis=-1):
    return jax.nn.softmax(x, axis=axis)

def _gelu(x):
    return jax.nn.gelu(x, approximate=True)

def _silu(x):
    return jax.nn.silu(x)

def _sigmoid(x):
    return jax.nn.sigmoid(x)

def _layernorm(x, axis=-1, eps=1e-05):
    m = jnp.mean(x, axis=axis, keepdims=True)
    v = jnp.var(x, axis=axis, keepdims=True)
    return (x - m) / jnp.sqrt(v + eps)

def _scatter_add(tgt, idx, src, axis=0):
    return tgt.at[idx].add(src)

def _segment_sum(src, seg, n):
    return jax.ops.segment_sum(src, seg, n)

class _Rng:

    def __init__(self, key):
        self._k = key

    def _next(self):
        self._k, sub = jax.random.split(self._k)
        return sub

    def normal(self, shape):
        return jax.random.normal(self._next(), shape, dtype=jnp.bfloat16)

    def randint(self, lo, hi, shape):
        return jax.random.randint(self._next(), shape, lo, hi, dtype=jnp.int32)

    def uniform(self, shape, lo=0.0, hi=1.0):
        return jax.random.uniform(self._next(), shape, jnp.bfloat16, lo, hi)

    def permutation(self, n):
        return jax.random.permutation(self._next(), n)
kernel_name = 'sequential_preLN__ssm_conv_s4__mixer_gmlp__prompt'

def _fwd_setup_inputs():
    _rng = _Rng(jax.random.key(int.from_bytes(__import__("os").urandom(4), "little")))
    _w = lambda a: (lambda t: t.astype(jnp.bfloat16) if jnp.issubdtype(t.dtype, jnp.floating) else t)(jnp.asarray(a))

    def _A_setup():
        B, L, D, N = (1, 2048, 576, 128)
        A_re = -jnp.exp((lambda *s: _rng.normal(s) * 0.05)(D, N))
        A_im = jnp.pi * (lambda *s: _rng.normal(s) * 0.05)(D, N)
        B_re = (lambda *s: _rng.normal(s) * 0.05)(D, N)
        B_im = (lambda *s: _rng.normal(s) * 0.05)(D, N)
        C_re = (lambda *s: _rng.normal(s) * 0.05)(D, N)
        C_im = (lambda *s: _rng.normal(s) * 0.05)(D, N)
        log_dt = (lambda *s: _rng.normal(s) * 0.05)(D) * 0.5 - 4.0
        Dskip = (lambda *s: _rng.normal(s) * 0.05)(D)
        return {'u': _w((lambda *s: _rng.normal(s) * 0.05)(B, L, D)), 'A_re': _w(A_re), 'A_im': _w(A_im), 'B_re': _w(B_re), 'B_im': _w(B_im), 'C_re': _w(C_re), 'C_im': _w(C_im), 'log_dt': _w(log_dt), 'Dskip': _w(Dskip)}
    _A_in = _A_setup()

    def _B_setup():
        B, S, D, F = (1, 2048, 576, 4608)
        Fh = F // 2
        return {'x': _w((lambda *s: _rng.normal(s) * 0.05)(B, S, D)), 'w_in': _w((lambda *s: _rng.normal(s) * 0.05)(D, 2 * Fh)), 'w_sp': _w(0.01 * (lambda *s: _rng.normal(s) * 0.05)(S, S)), 'b_sp': _w(1.0 + 0.01 * (lambda *s: _rng.normal(s) * 0.05)(S)), 'w_out': _w((lambda *s: _rng.normal(s) * 0.05)(Fh, D))}
    _B_in = _B_setup()
    return {'A_u': _A_in['u'], 'A_A_re': _A_in['A_re'], 'A_A_im': _A_in['A_im'], 'A_B_re': _A_in['B_re'], 'A_B_im': _A_in['B_im'], 'A_C_re': _A_in['C_re'], 'A_C_im': _A_in['C_im'], 'A_log_dt': _A_in['log_dt'], 'A_Dskip': _A_in['Dskip'], 'B_x': _B_in['x'], 'B_w_in': _B_in['w_in'], 'B_w_sp': _B_in['w_sp'], 'B_b_sp': _B_in['b_sp'], 'B_w_out': _B_in['w_out']}

def _fwd_reference(A_u, A_A_re, A_A_im, A_B_re, A_B_im, A_C_re, A_C_im, A_log_dt, A_Dskip, B_x, B_w_in, B_w_sp, B_b_sp, B_w_out):

    def _A_ref(u, A_re, A_im, B_re, B_im, C_re, C_im, log_dt, Dskip):
        Bsz, L, D = u.shape
        dt = jnp.exp(log_dt)[:, None]
        A = A_re + 1j * A_im
        Bc = B_re + 1j * B_im
        Cc = C_re + 1j * C_im
        logdA = dt * A
        dB = dt * Bc
        l = (lambda x, dt: x.astype(dt))(jnp.arange(L), A_re.dtype)
        P = jnp.exp(logdA[:, :, None] * l[None, None, :])
        K = jnp.einsum('dn,dnl,dn->dl', Cc, P, dB).real
        L2 = 2 * L
        Kp = jnp.pad(K, ((0, 0), (0, L)))
        up = (lambda x, *d: x.transpose(*d))(u, 0, 2, 1)
        up = jnp.pad(up, ((0, 0), (0, 0), (0, L)))
        Kf = (lambda x, axes=(-2, -1): jnp.fft.rfft2(x.astype(jnp.float32), axes=axes))(Kp[:, None, :], axes=(-2, -1))
        Uf = (lambda x, axes=(-2, -1): jnp.fft.rfft2(x.astype(jnp.float32), axes=axes))(up[:, :, None, :], axes=(-2, -1))
        Yf = Uf * Kf[None, :, :, :]
        y = (lambda x, s, axes=(-2, -1): jnp.fft.irfft2(x, s=s, axes=axes).astype(jnp.bfloat16))(Yf, (1, L2), axes=(-2, -1))[:, :, 0, :L]
        y = (lambda x, *d: x.transpose(*d))(y, 0, 2, 1) + u * Dskip[None, None, :]
        return y

    def _B_ref(x, w_in, w_sp, b_sp, w_out):
        B, S, D = x.shape
        F = w_in.shape[-1]
        Fh = F // 2
        z = _gelu(jnp.einsum('bsd,df->bsf', x, w_in))
        z1 = z[..., :Fh].copy()
        z2 = _layernorm(z[..., Fh:], axis=-1)
        g = jnp.einsum('ts,bsf->btf', w_sp, z2) + b_sp[None, :, None]
        return jnp.einsum('bsf,fd->bsd', z1 * g, w_out)
    x = A_u
    h = x + _A_ref(_layernorm(x, axis=-1), A_A_re, A_A_im, A_B_re, A_B_im, A_C_re, A_C_im, A_log_dt, A_Dskip)
    h2 = h + _B_ref(_layernorm(h, axis=-1), B_w_in, B_w_sp, B_b_sp, B_w_out)
    return h2

def setup_inputs():
    _inp = _fwd_setup_inputs()
    _gk = jax.random.fold_in(jax.random.key(int.from_bytes(__import__("os").urandom(4), "little")), 2 ** 31 - 1)
    _shapes = [[1, 2048, 576]]
    _dtypes = ['bfloat16']
    _gks = jax.random.split(_gk, len(_shapes))
    _gs = [jax.random.normal(k, s, dtype=jnp.dtype(d)) * 0.05 for k, s, d in zip(_gks, _shapes, _dtypes)]
    _inp['grad_out'] = _gs[0]
    return _inp

def reference(A_u, A_A_re, A_A_im, A_B_re, A_B_im, A_C_re, A_C_im, A_log_dt, A_Dskip, B_w_in, B_w_sp, B_b_sp, B_w_out, B_x, grad_out):
    _const = dict(B_x=B_x)

    def _f(*_d):
        return _fwd_reference(**{'A_u': _d[0], 'A_A_re': _d[1], 'A_A_im': _d[2], 'A_B_re': _d[3], 'A_B_im': _d[4], 'A_C_re': _d[5], 'A_C_im': _d[6], 'A_log_dt': _d[7], 'A_Dskip': _d[8], 'B_w_in': _d[9], 'B_w_sp': _d[10], 'B_b_sp': _d[11], 'B_w_out': _d[12], **_const})
    _out, _vjp = jax.vjp(_f, A_u, A_A_re, A_A_im, A_B_re, A_B_im, A_C_re, A_C_im, A_log_dt, A_Dskip, B_w_in, B_w_sp, B_b_sp, B_w_out)
    _grads = _vjp(grad_out)
    _out0 = jnp.asarray(_out)
    return (_out0, *[jnp.asarray(_g) for _g in _grads])
```

```python
import numpy as np
import jax
import jax.numpy as jnp
import jax.experimental.pallas as pl
import jax.experimental.pallas.tpu as pltpu

S, D, N, F = 2048, 576, 128, 4608
FH = F // 2
Q = 128
NB = S // Q
TM = 256
NT = S // TM
KU = 768
EPS = 1e-5
f32, bf16 = jnp.float32, jnp.bfloat16
SEGS = ((0, 1, 32, 0), (256, 2, 16, 256), (512, 4, 16, 384), (1024, 8, 17, 512))


def _split(a):
    a = np.asarray(a, np.float32)
    hi = a.astype(jnp.bfloat16)
    lo = (a - hi.astype(np.float32)).astype(jnp.bfloat16)
    return hi, lo


def _consts():
    fr = (np.arange(Q) + 0.5)[:, None]
    th = 2.0 * np.pi * fr * np.arange(2 * Q)[None, :] / (2 * Q)
    fm = np.concatenate([np.cos(th[:, :Q]), -np.sin(th[:, :Q])], 0)
    gm = np.concatenate([np.cos(th).T, -np.sin(th).T], 1) * (2.0 / (2 * Q))
    uniq = np.concatenate([s0 + st * np.arange(8 * nk) for s0, st, nk, _ in SEGS])
    lb = np.arange(S).astype(jnp.bfloat16).astype(np.int64)
    pos = {int(v): i for i, v in enumerate(uniq)}
    u_of_l = np.array([pos[int(v)] for v in lb])
    offs = [int(u_of_l[j * Q]) for j in range(NB)]
    fs = np.zeros((NB, 2 * Q, Q))
    for j in range(NB):
        assert offs[j] % 8 == 0
        sel = np.zeros((Q, Q))
        sel[np.arange(Q), u_of_l[j * Q:(j + 1) * Q] - offs[j]] = 1.0
        fs[j] = fm @ sel
    lcol = np.zeros((KU, 1), np.float32)
    lcol[:len(uniq), 0] = uniq
    mats = [fm, fm.T, gm, gm.T, fs, fs.transpose(0, 2, 1)]
    out = []
    for m in mats:
        out.extend(_split(m))
    return out, offs, lcol


_CM, _OFFS, _LCOL = _consts()


def _dot(a, b):
    return jnp.dot(a, b, preferred_element_type=f32)


def _dot_nt(a, b):
    return jax.lax.dot_general(a, b, (((1,), (1,)), ((), ())), preferred_element_type=f32)


def _dot_tn(a, b):
    return jax.lax.dot_general(a, b, (((0,), (0,)), ((), ())), preferred_element_type=f32)


def _dot2(ah, al, xb):
    return _dot(ah, xb) + _dot(al, xb)


def _dot3(ah, al, x):
    xh = x.astype(bf16)
    xl = (x - xh.astype(f32)).astype(bf16)
    return _dot(ah, xh) + (_dot(ah, xl) + _dot(al, xh))


def _ln(x):
    m = jnp.mean(x, axis=-1, keepdims=True)
    c = x - m
    v = jnp.mean(c * c, axis=-1, keepdims=True)
    r = jax.lax.rsqrt(v + EPS)
    return c * r, r


def _ln_bwd(dy, xh, r):
    return r * (dy - jnp.mean(dy, axis=-1, keepdims=True)
                - xh * jnp.mean(dy * xh, axis=-1, keepdims=True))


_GC = 0.7978845608028654


def _gelu(p):
    return 0.5 * p * (1.0 + jnp.tanh(_GC * (p + 0.044715 * p * p * p)))


def _gelu_both(p):
    t = jnp.tanh(_GC * (p + 0.044715 * p * p * p))
    z = 0.5 * p * (1.0 + t)
    dz = 0.5 * (1.0 + t) + 0.5 * p * (1.0 - t * t) * _GC * (1.0 + 3 * 0.044715 * p * p)
    return z, dz


def _cmul(ar, ai, br, bi):
    return ar * br - ai * bi, ar * bi + ai * br


def _kernel(x_ref, go_ref, are_ref, aim_ref, bre_ref, bim_ref, cre_ref, cim_ref,
            ldt_ref, dsk_ref, win_ref, wsp_ref, wspt_ref, bsp_ref, wout_ref, lcol_ref,
            fmh, fml, fmth, fmtl, gmh, gml, gmth, gmtl, fsh, fsl, fsth, fstl,
            h2_ref, dx_ref, dare_ref, daim_ref, dbre_ref, dbim_ref, dcre_ref, dcim_ref,
            dldt_ref, ddsk_ref, dwin_hbm, dwsp_hbm, dbsp_ref, dwout_ref,
            xn_s, h_s, dh_s, kf_s, ku_s, sem):
    dt = jnp.exp(ldt_ref[...].astype(f32)).astype(bf16).astype(f32)
    dsk = dsk_ref[...].astype(f32)
    are = are_ref[...].astype(f32)
    aim = aim_ref[...].astype(f32)
    rio = jax.lax.broadcasted_iota(jnp.int32, (8, D), 0)

    lre, lim = dt * are, dt * aim
    pw = {}

    def fill_tables(pwr_s, pwi_s):
        pw['r'], pw['i'] = pwr_s, pwi_s
        for k in range(12):
            e = jnp.exp(lre * float(2 ** k))
            pwr_s[k] = e * jnp.cos(lim * float(2 ** k))
            pwi_s[k] = e * jnp.sin(lim * float(2 ** k))

    def prow(k, n):
        return pw['r'][k, pl.ds(n, 1), :], pw['i'][k, pl.ds(n, 1), :]

    def bits_block(k0, n):
        outr = outi = None
        for b in range(3):
            pr, pi = prow(k0 + b, n)
            on = ((rio >> b) & 1) == 1
            tr, ti = jnp.where(on, pr, 1.0), jnp.where(on, pi, 0.0)
            if outr is None:
                outr, outi = tr, ti
            else:
                outr, outi = _cmul(outr, outi, tr, ti)
        return outr, outi

    def seg_tables(seg, n):
        s0, st, nk, _ = seg
        ks = st.bit_length() - 1
        er, ei = bits_block(ks, n)
        g0r, g0i = bits_block(ks + 3, n)
        if s0:
            pr, pi = prow(s0.bit_length() - 1, n)
            g0r, g0i = _cmul(g0r, g0i, pr, pi)
        gr, gi = [g0r], [g0i]
        pr, pi = prow(ks + 6, n)
        for _b in range((nk + 7) // 8 - 1):
            a, b = _cmul(gr[-1], gi[-1], pr, pi)
            gr.append(a)
            gi.append(b)
        gr = jnp.concatenate(gr, 0)[:nk].reshape(nk, 1, D)
        gi = jnp.concatenate(gi, 0)[:nk].reshape(nk, 1, D)
        return er, ei, gr, gi

    def cb_row(n):
        br = dt * bre_ref[pl.ds(n, 1), :].astype(f32)
        bi = dt * bim_ref[pl.ds(n, 1), :].astype(f32)
        cr = cre_ref[pl.ds(n, 1), :].astype(f32)
        ci = cim_ref[pl.ds(n, 1), :].astype(f32)
        return br, bi, cr, ci

    ku_s[...] = jnp.zeros((KU, D), f32)

    def kgen(n, c):
        br, bi, cr, ci = cb_row(n)
        wr, wi = _cmul(cr, ci, br, bi)
        for seg in SEGS:
            _, _, nk, ro = seg
            er, ei, gr, gi = seg_tables(seg, n)
            cer, cei = _cmul(er, ei, wr, wi)
            t = cer[None] * gr - cei[None] * gi
            ku_s[ro:ro + 8 * nk, :] += t.reshape(8 * nk, D)
        return c

    def sc_gen(pa, pb):
        fill_tables(pa, pb)
        jax.lax.fori_loop(0, N, kgen, 0)
    pl.run_scoped(sc_gen, pltpu.VMEM((12, N, D), f32), pltpu.VMEM((12, N, D), f32))

    for j in range(NB):
        kf_s[j] = _dot3(fsh[j], fsl[j], ku_s[_OFFS[j]:_OFFS[j] + Q, :])

    def fwd_a(uf_s):
        def p1(a, c):
            rows = pl.ds(pl.multiple_of(a * Q, Q), Q)
            xn, _ = _ln(x_ref[rows, :].astype(f32))
            xn = xn.astype(bf16)
            xn_s[rows, :] = xn
            uf_s[a] = _dot2(fmh[...], fml[...], xn)
            return c
        jax.lax.fori_loop(0, NB, p1, 0)

        def p2(a, prev):
            def inner(j, acc):
                kf = kf_s[j]
                uf = uf_s[a - j]
                pr, pi = _cmul(kf[:Q], kf[Q:], uf[:Q], uf[Q:])
                return acc[0] + pr, acc[1] + pi
            z0 = jnp.zeros((Q, D), f32)
            wr, wi = jax.lax.fori_loop(0, a + 1, inner, (z0, z0))
            w = _dot3(gmh[...], gml[...], jnp.concatenate([wr, wi], 0))
            rows = pl.ds(pl.multiple_of(a * Q, Q), Q)
            y = (w[:Q] + prev).astype(bf16).astype(f32)
            y2 = (y + (xn_s[rows, :].astype(f32) * dsk).astype(bf16).astype(f32)).astype(bf16)
            h_s[rows, :] = (x_ref[rows, :].astype(f32) + y2.astype(f32)).astype(bf16)
            return w[Q:]
        jax.lax.fori_loop(0, NB, p2, jnp.zeros((Q, D), f32))
    pl.run_scoped(fwd_a, pltpu.VMEM((NB, 2 * Q, D), f32))

    def phase_b(hn_s, zp_s, z2_s, dg_s, dwo_s, st_s, st2_s):
        def l1(i, c):
            rows = pl.ds(pl.multiple_of(i * TM, TM), TM)
            hn, _ = _ln(h_s[rows, :].astype(f32))
            hn = hn.astype(bf16)
            hn_s[rows, :] = hn
            zp = _dot(hn, win_ref[...]).astype(bf16)
            zp_s[rows, :] = zp
            z2 = _gelu(zp[:, FH:].astype(f32)).astype(bf16).astype(f32)
            z2_s[rows, :] = _ln(z2)[0].astype(bf16)
            return c
        jax.lax.fori_loop(0, NT, l1, 0)
        dwo_s[...] = jnp.zeros((FH, D), f32)

        def l2(i, c):
            rows = pl.ds(pl.multiple_of(i * TM, TM), TM)
            g = _dot(wsp_ref[rows, :], z2_s[...]) + bsp_ref[rows, :].astype(f32)
            g = g.astype(bf16).astype(f32)
            z1, dz1 = _gelu_both(zp_s[rows, :FH].astype(f32))
            z1 = z1.astype(bf16).astype(f32)
            zg = (z1 * g).astype(bf16)
            o = _dot(zg, wout_ref[...]).astype(bf16).astype(f32)
            h2_ref[rows, :] = (h_s[rows, :].astype(f32) + o).astype(bf16)
            go = go_ref[rows, :]
            dzg = _dot_nt(go, wout_ref[...]).astype(bf16).astype(f32)
            dwo_s[...] += _dot_tn(zg, go)
            zp_s[rows, :FH] = (dzg * g * dz1).astype(bf16)
            dg = dzg * z1
            dbsp_ref[rows, :] = jnp.sum(dg, axis=-1, keepdims=True).astype(bf16)
            dg = dg.astype(bf16)
            dg_s[rows, :] = dg
            st_s[...] = _dot_nt(dg, z2_s[...]).astype(bf16)
            cp = pltpu.make_async_copy(st_s, dwsp_hbm.at[rows, :], sem.at[0])
            cp.start()
            cp.wait()
            return c
        jax.lax.fori_loop(0, NT, l2, 0)
        dwout_ref[...] = dwo_s[...].astype(bf16)

        def l3(i, c):
            rows = pl.ds(pl.multiple_of(i * TM, TM), TM)
            cp = pltpu.make_async_copy(wspt_ref.at[rows, :], st_s, sem.at[0])
            cp.start()
            cp.wait()
            dz2n = _dot(st_s[...], dg_s[...])
            z2, dz2 = _gelu_both(zp_s[rows, FH:].astype(f32))
            z2h, r2 = _ln(z2.astype(bf16).astype(f32))
            zp_s[rows, FH:] = (_ln_bwd(dz2n, z2h, r2) * dz2).astype(bf16)
            dhn = _dot_nt(zp_s[rows, :], win_ref[...])
            hh, r1 = _ln(h_s[rows, :].astype(f32))
            dh_s[rows, :] = (go_ref[rows, :].astype(f32) + _ln_bwd(dhn, hh, r1)).astype(bf16)
            return c
        jax.lax.fori_loop(0, NT, l3, 0)

        for cblk in range(F // 512):
            cs = slice(cblk * 512, (cblk + 1) * 512)
            st2_s[...] = _dot_tn(hn_s[...], zp_s[:, cs]).astype(bf16)
            cp = pltpu.make_async_copy(st2_s, dwin_hbm.at[:, cs], sem.at[1])
            cp.start()
            cp.wait()
    pl.run_scoped(phase_b, pltpu.VMEM((S, D), bf16), pltpu.VMEM((S, F), bf16),
                  pltpu.VMEM((S, FH), bf16), pltpu.VMEM((S, FH), bf16),
                  pltpu.VMEM((FH, D), f32), pltpu.VMEM((TM, S), bf16),
                  pltpu.VMEM((D, 512), bf16))

    def bwd_a(uf_s, dw_s):
        ku_s[...] = jnp.zeros((KU, D), f32)

        def q1(a, acc):
            rows = pl.ds(pl.multiple_of(a * Q, Q), Q)
            nrows = pl.ds(pl.multiple_of(jnp.minimum(a + 1, NB - 1) * Q, Q), Q)
            dh = dh_s[rows, :]
            nxt = jnp.where(a + 1 < NB, dh_s[nrows, :], jnp.zeros((Q, D), bf16))
            dw_s[a] = _dot2(gmth[...], gmtl[...], jnp.concatenate([dh, nxt], 0))
            xn = xn_s[rows, :]
            uf_s[a] = _dot2(fmh[...], fml[...], xn)
            return acc + jnp.sum(dh.astype(f32) * xn.astype(f32), axis=0, keepdims=True)
        ddsk_ref[...] = jax.lax.fori_loop(0, NB, q1, jnp.zeros((1, D), f32)).astype(bf16)

        def corr(b, other):
            def inner(a, acc):
                dw = dw_s[a]
                o = other[a - b]
                return (acc[0] + dw[:Q] * o[:Q] + dw[Q:] * o[Q:],
                        acc[1] + dw[Q:] * o[:Q] - dw[:Q] * o[Q:])
            z0 = jnp.zeros((Q, D), f32)
            r, i = jax.lax.fori_loop(b, NB, inner, (z0, z0))
            return jnp.concatenate([r, i], 0)

        def q2(b, c):
            rows = pl.ds(pl.multiple_of(b * Q, Q), Q)
            dxn = _dot3(fmth[...], fmtl[...], corr(b, kf_s))
            dh = dh_s[rows, :].astype(f32)
            xh, r = _ln(x_ref[rows, :].astype(f32))
            dx_ref[rows, :] = (dh + _ln_bwd(dxn + dh * dsk, xh, r)).astype(bf16)
            return c
        jax.lax.fori_loop(0, NB, q2, 0)

        for j in range(NB):
            ku_s[_OFFS[j]:_OFFS[j] + Q, :] += _dot3(fsth[j], fstl[j], corr(j, uf_s))
    pl.run_scoped(bwd_a, pltpu.VMEM((NB, 2 * Q, D), f32), pltpu.VMEM((NB, 2 * Q, D), f32))

    def kbwd(n, ddt):
        br, bi, cr, ci = cb_row(n)
        s0r = s0i = s1r = s1i = jnp.zeros((1, D), f32)
        for seg in SEGS:
            _, _, nk, ro = seg
            er, ei, gr, gi = seg_tables(seg, n)
            t = ku_s[ro:ro + 8 * nk, :]
            tl = (t * lcol_ref[ro:ro + 8 * nk, :]).reshape(nk, 8, D)
            t = t.reshape(nk, 8, D)
            a0r, a0i = _cmul(jnp.sum(t * gr, 0), jnp.sum(t * gi, 0), er, ei)
            a1r, a1i = _cmul(jnp.sum(tl * gr, 0), jnp.sum(tl * gi, 0), er, ei)
            s0r = s0r + jnp.sum(a0r, 0, keepdims=True)
            s0i = s0i + jnp.sum(a0i, 0, keepdims=True)
            s1r = s1r + jnp.sum(a1r, 0, keepdims=True)
            s1i = s1i + jnp.sum(a1i, 0, keepdims=True)
        row = pl.ds(n, 1)
        tr, ti = _cmul(br, bi, s0r, s0i)
        dcre_ref[row, :] = tr
        dcim_ref[row, :] = (-ti)
        tr, ti = _cmul(cr, ci, s0r, s0i)
        dbre_ref[row, :] = (dt * tr)
        dbim_ref[row, :] = (-dt * ti)
        b0r = bre_ref[row, :].astype(f32)
        b0i = bim_ref[row, :].astype(f32)
        wr, wi = _cmul(cr, ci, br, bi)
        gre, gim = _cmul(wr, wi, s1r, s1i)
        gim = -gim
        dare_ref[row, :] = (dt * gre)
        daim_ref[row, :] = (dt * gim)
        return (ddt + are_ref[row, :].astype(f32) * gre + aim_ref[row, :].astype(f32) * gim
                + tr * b0r - ti * b0i)

    def sc_bwd(pa, pb):
        fill_tables(pa, pb)
        ddt = jax.lax.fori_loop(0, N, kbwd, jnp.zeros((1, D), f32))
        dldt_ref[...] = (ddt * dt).astype(bf16)
    pl.run_scoped(sc_bwd, pltpu.VMEM((12, N, D), f32), pltpu.VMEM((12, N, D), f32))


@jax.jit
def pallas_sequential_preLN__ssm_conv_s4__mixer_gmlp__prompt_kernel(
    A_u, A_A_re, A_A_im, A_B_re, A_B_im, A_C_re, A_C_im, A_log_dt, A_Dskip,
    B_x, B_w_in, B_w_sp, B_b_sp, B_w_out, grad_out,
):
    vm = pl.BlockSpec(memory_space=pltpu.VMEM)
    hbm = pl.BlockSpec(memory_space=pl.ANY)
    sd = lambda *s: jax.ShapeDtypeStruct(s, bf16)
    ins = [A_u.reshape(S, D), grad_out.reshape(S, D), A_A_re.T.astype(f32), A_A_im.T.astype(f32), A_B_re.T.astype(f32), A_B_im.T.astype(f32),
           A_C_re.T.astype(f32), A_C_im.T.astype(f32), A_log_dt.reshape(1, D), A_Dskip.reshape(1, D), B_w_in, B_w_sp,
           B_w_sp.T, B_b_sp.reshape(S, 1), B_w_out, jnp.asarray(_LCOL)]
    ins += [jnp.asarray(m) for m in _CM]
    outs = pl.pallas_call(
        _kernel,
        out_shape=[sd(S, D), sd(S, D)] + [jax.ShapeDtypeStruct((N, D), f32)] * 6 + [sd(1, D), sd(1, D), sd(D, F),
                                                            sd(S, S), sd(S, 1), sd(FH, D)],
        in_specs=[vm] * 12 + [hbm] + [vm] * (len(ins) - 13),
        out_specs=[vm] * 10 + [hbm, hbm, vm, vm],
        scratch_shapes=[pltpu.VMEM((S, D), bf16), pltpu.VMEM((S, D), bf16),
                        pltpu.VMEM((S, D), bf16), pltpu.VMEM((NB, 2 * Q, D), f32),
                        pltpu.VMEM((KU, D), f32), pltpu.SemaphoreType.DMA((2,))],
        compiler_params=pltpu.CompilerParams(vmem_limit_bytes=127 * 1024 * 1024),
    )(*ins)
    (h2, dx, dare, daim, dbre, dbim, dcre, dcim, dldt, ddsk, dwin, dwsp, dbsp, dwout) = outs
    return (h2.reshape(1, S, D), dx.reshape(1, S, D), *[t.T.astype(bf16) for t in (dare, daim, dbre, dbim, dcre, dcim)],
            dldt.reshape(D), ddsk.reshape(D), dwin, dwsp, dbsp.reshape(S), dwout)
```

```python
import numpy as np
import jax
import jax.numpy as jnp
import jax.experimental.pallas as pl
import jax.experimental.pallas.tpu as pltpu

S, D, N, F = 2048, 576, 128, 4608
FH = F // 2
Q = 128
NB = S // Q
TM = 256
NT = S // TM
KU = 768
EPS = 1e-5
f32, bf16 = jnp.float32, jnp.bfloat16
SEGS = ((0, 1, 32, 0), (256, 2, 16, 256), (512, 4, 16, 384), (1024, 8, 17, 512))


def _split(a):
    a = np.asarray(a, np.float32)
    hi = a.astype(jnp.bfloat16)
    lo = (a - hi.astype(np.float32)).astype(jnp.bfloat16)
    return hi, lo


def _consts():
    fr = (np.arange(Q) + 0.5)[:, None]
    th = 2.0 * np.pi * fr * np.arange(2 * Q)[None, :] / (2 * Q)
    fm = np.concatenate([np.cos(th[:, :Q]), -np.sin(th[:, :Q])], 0)
    gm = np.concatenate([np.cos(th).T, -np.sin(th).T], 1) * (2.0 / (2 * Q))
    uniq = np.concatenate([s0 + st * np.arange(8 * nk) for s0, st, nk, _ in SEGS])
    lb = np.arange(S).astype(jnp.bfloat16).astype(np.int64)
    pos = {int(v): i for i, v in enumerate(uniq)}
    u_of_l = np.array([pos[int(v)] for v in lb])
    offs = [int(u_of_l[j * Q]) for j in range(NB)]
    fs = np.zeros((NB, 2 * Q, Q))
    for j in range(NB):
        assert offs[j] % 8 == 0
        sel = np.zeros((Q, Q))
        sel[np.arange(Q), u_of_l[j * Q:(j + 1) * Q] - offs[j]] = 1.0
        fs[j] = fm @ sel
    lcol = np.zeros((KU, 1), np.float32)
    lcol[:len(uniq), 0] = uniq
    mats = [fm, fm.T, gm, gm.T, fs, fs.transpose(0, 2, 1)]
    out = []
    for m in mats:
        out.extend(_split(m))
    return out, offs, lcol


_CM, _OFFS, _LCOL = _consts()


def _dot(a, b):
    return jnp.dot(a, b, preferred_element_type=f32)


def _dot_nt(a, b):
    return jax.lax.dot_general(a, b, (((1,), (1,)), ((), ())), preferred_element_type=f32)


def _dot_tn(a, b):
    return jax.lax.dot_general(a, b, (((0,), (0,)), ((), ())), preferred_element_type=f32)


def _dot2(ah, al, xb):
    return _dot(ah, xb) + _dot(al, xb)


def _dot3(ah, al, x):
    xh = x.astype(bf16)
    xl = (x - xh.astype(f32)).astype(bf16)
    return _dot(ah, xh) + (_dot(ah, xl) + _dot(al, xh))


def _ln(x):
    m = jnp.mean(x, axis=-1, keepdims=True)
    c = x - m
    v = jnp.mean(c * c, axis=-1, keepdims=True)
    r = jax.lax.rsqrt(v + EPS)
    return c * r, r


def _ln_bwd(dy, xh, r):
    return r * (dy - jnp.mean(dy, axis=-1, keepdims=True)
                - xh * jnp.mean(dy * xh, axis=-1, keepdims=True))


_GC = 0.7978845608028654


def _gelu(p):
    return 0.5 * p * (1.0 + jnp.tanh(_GC * (p + 0.044715 * p * p * p)))


def _gelu_both(p):
    t = jnp.tanh(_GC * (p + 0.044715 * p * p * p))
    z = 0.5 * p * (1.0 + t)
    dz = 0.5 * (1.0 + t) + 0.5 * p * (1.0 - t * t) * _GC * (1.0 + 3 * 0.044715 * p * p)
    return z, dz


def _cmul(ar, ai, br, bi):
    return ar * br - ai * bi, ar * bi + ai * br


def _kernel(x_ref, go_ref, are_ref, aim_ref, bre_ref, bim_ref, cre_ref, cim_ref,
            ldt_ref, dsk_ref, win_ref, wsp_ref, bsp_ref, wout_ref, lcol_ref,
            fmh, fml, fmth, fmtl, gmh, gml, gmth, gmtl, fsh, fsl, fsth, fstl,
            h2_ref, dx_ref, dare_ref, daim_ref, dbre_ref, dbim_ref, dcre_ref, dcim_ref,
            dldt_ref, ddsk_ref, dwin_hbm, dwsp_hbm, dbsp_ref, dwout_ref,
            xn_s, h_s, dh_s, kf_s, ku_s, sem):
    dt = jnp.exp(ldt_ref[...].astype(f32)).astype(bf16).astype(f32)
    dsk = dsk_ref[...].astype(f32)
    are = are_ref[...].astype(f32)
    aim = aim_ref[...].astype(f32)
    rio = jax.lax.broadcasted_iota(jnp.int32, (8, D), 0)

    lre, lim = dt * are, dt * aim
    pw = {}

    def fill_tables(pwr_s, pwi_s):
        pw['r'], pw['i'] = pwr_s, pwi_s
        for k in range(12):
            e = jnp.exp(lre * float(2 ** k))
            pwr_s[k] = e * jnp.cos(lim * float(2 ** k))
            pwi_s[k] = e * jnp.sin(lim * float(2 ** k))

    def prow(k, n):
        return pw['r'][k, pl.ds(n, 1), :], pw['i'][k, pl.ds(n, 1), :]

    def bits_block(k0, n):
        outr = outi = None
        for b in range(3):
            pr, pi = prow(k0 + b, n)
            on = ((rio >> b) & 1) == 1
            tr, ti = jnp.where(on, pr, 1.0), jnp.where(on, pi, 0.0)
            if outr is None:
                outr, outi = tr, ti
            else:
                outr, outi = _cmul(outr, outi, tr, ti)
        return outr, outi

    def seg_tables(seg, n):
        s0, st, nk, _ = seg
        ks = st.bit_length() - 1
        er, ei = bits_block(ks, n)
        g0r, g0i = bits_block(ks + 3, n)
        if s0:
            pr, pi = prow(s0.bit_length() - 1, n)
            g0r, g0i = _cmul(g0r, g0i, pr, pi)
        gr, gi = [g0r], [g0i]
        pr, pi = prow(ks + 6, n)
        for _b in range((nk + 7) // 8 - 1):
            a, b = _cmul(gr[-1], gi[-1], pr, pi)
            gr.append(a)
            gi.append(b)
        gr = jnp.concatenate(gr, 0)[:nk].reshape(nk, 1, D)
        gi = jnp.concatenate(gi, 0)[:nk].reshape(nk, 1, D)
        return er, ei, gr, gi

    def cb_row(n):
        br = dt * bre_ref[pl.ds(n, 1), :].astype(f32)
        bi = dt * bim_ref[pl.ds(n, 1), :].astype(f32)
        cr = cre_ref[pl.ds(n, 1), :].astype(f32)
        ci = cim_ref[pl.ds(n, 1), :].astype(f32)
        return br, bi, cr, ci

    ku_s[...] = jnp.zeros((KU, D), f32)

    def kgen(n, c):
        br, bi, cr, ci = cb_row(n)
        wr, wi = _cmul(cr, ci, br, bi)
        for seg in SEGS:
            _, _, nk, ro = seg
            er, ei, gr, gi = seg_tables(seg, n)
            cer, cei = _cmul(er, ei, wr, wi)
            t = cer[None] * gr - cei[None] * gi
            ku_s[ro:ro + 8 * nk, :] += t.reshape(8 * nk, D)
        return c

    def sc_gen(pa, pb):
        fill_tables(pa, pb)
        jax.lax.fori_loop(0, N, kgen, 0)
    pl.run_scoped(sc_gen, pltpu.VMEM((12, N, D), f32), pltpu.VMEM((12, N, D), f32))

    for j in range(NB):
        kf_s[j] = _dot3(fsh[j], fsl[j], ku_s[_OFFS[j]:_OFFS[j] + Q, :])

    def fwd_a(uf_s):
        def p1(a, c):
            rows = pl.ds(pl.multiple_of(a * Q, Q), Q)
            xn, _ = _ln(x_ref[rows, :].astype(f32))
            xn = xn.astype(bf16)
            xn_s[rows, :] = xn
            uf_s[a] = _dot2(fmh[...], fml[...], xn)
            return c
        jax.lax.fori_loop(0, NB, p1, 0)

        def p2(a, prev):
            def inner(j, acc):
                kf = kf_s[j]
                uf = uf_s[a - j]
                pr, pi = _cmul(kf[:Q], kf[Q:], uf[:Q], uf[Q:])
                return acc[0] + pr, acc[1] + pi
            z0 = jnp.zeros((Q, D), f32)
            wr, wi = jax.lax.fori_loop(0, a + 1, inner, (z0, z0))
            w = _dot3(gmh[...], gml[...], jnp.concatenate([wr, wi], 0))
            rows = pl.ds(pl.multiple_of(a * Q, Q), Q)
            y = (w[:Q] + prev).astype(bf16).astype(f32)
            y2 = (y + (xn_s[rows, :].astype(f32) * dsk).astype(bf16).astype(f32)).astype(bf16)
            h_s[rows, :] = (x_ref[rows, :].astype(f32) + y2.astype(f32)).astype(bf16)
            return w[Q:]
        jax.lax.fori_loop(0, NB, p2, jnp.zeros((Q, D), f32))
    pl.run_scoped(fwd_a, pltpu.VMEM((NB, 2 * Q, D), f32))

    def phase_b(hn_s, zp_s, z2_s, dg_s, dwo_s, st_s, st2_s):
        def l1(i, c):
            rows = pl.ds(pl.multiple_of(i * TM, TM), TM)
            hn, _ = _ln(h_s[rows, :].astype(f32))
            hn = hn.astype(bf16)
            hn_s[rows, :] = hn
            zp = _dot(hn, win_ref[...]).astype(bf16)
            zp_s[rows, :] = zp
            z2 = _gelu(zp[:, FH:].astype(f32)).astype(bf16).astype(f32)
            z2_s[rows, :] = _ln(z2)[0].astype(bf16)
            return c
        jax.lax.fori_loop(0, NT, l1, 0)
        dwo_s[...] = jnp.zeros((FH, D), f32)

        def l2(i, c):
            rows = pl.ds(pl.multiple_of(i * TM, TM), TM)
            g = _dot(wsp_ref[rows, :], z2_s[...]) + bsp_ref[rows, :].astype(f32)
            g = g.astype(bf16).astype(f32)
            z1, dz1 = _gelu_both(zp_s[rows, :FH].astype(f32))
            z1 = z1.astype(bf16).astype(f32)
            zg = (z1 * g).astype(bf16)
            o = _dot(zg, wout_ref[...]).astype(bf16).astype(f32)
            h2_ref[rows, :] = (h_s[rows, :].astype(f32) + o).astype(bf16)
            go = go_ref[rows, :]
            dzg = _dot_nt(go, wout_ref[...]).astype(bf16).astype(f32)
            dwo_s[...] += _dot_tn(zg, go)
            zp_s[rows, :FH] = (dzg * g * dz1).astype(bf16)
            dg = dzg * z1
            dbsp_ref[rows, :] = jnp.sum(dg, axis=-1, keepdims=True).astype(bf16)
            dg = dg.astype(bf16)
            dg_s[rows, :] = dg
            st_s[...] = _dot_nt(dg, z2_s[...]).astype(bf16)
            cp = pltpu.make_async_copy(st_s, dwsp_hbm.at[rows, :], sem.at[0])
            cp.start()
            cp.wait()
            return c
        jax.lax.fori_loop(0, NT, l2, 0)
        dwout_ref[...] = dwo_s[...].astype(bf16)

        def l3(i, c):
            rows = pl.ds(pl.multiple_of(i * TM, TM), TM)
            dz2n = _dot_tn(wsp_ref[:, rows], dg_s[...])
            z2, dz2 = _gelu_both(zp_s[rows, FH:].astype(f32))
            z2h, r2 = _ln(z2.astype(bf16).astype(f32))
            zp_s[rows, FH:] = (_ln_bwd(dz2n, z2h, r2) * dz2).astype(bf16)
            dhn = _dot_nt(zp_s[rows, :], win_ref[...])
            hh, r1 = _ln(h_s[rows, :].astype(f32))
            dh_s[rows, :] = (go_ref[rows, :].astype(f32) + _ln_bwd(dhn, hh, r1)).astype(bf16)
            return c
        jax.lax.fori_loop(0, NT, l3, 0)

        for cblk in range(F // 512):
            cs = slice(cblk * 512, (cblk + 1) * 512)
            st2_s[...] = _dot_tn(hn_s[...], zp_s[:, cs]).astype(bf16)
            cp = pltpu.make_async_copy(st2_s, dwin_hbm.at[:, cs], sem.at[1])
            cp.start()
            cp.wait()
    pl.run_scoped(phase_b, pltpu.VMEM((S, D), bf16), pltpu.VMEM((S, F), bf16),
                  pltpu.VMEM((S, FH), bf16), pltpu.VMEM((S, FH), bf16),
                  pltpu.VMEM((FH, D), f32), pltpu.VMEM((TM, S), bf16),
                  pltpu.VMEM((D, 512), bf16))

    def bwd_a(uf_s, dw_s):
        ku_s[...] = jnp.zeros((KU, D), f32)

        def q1(a, acc):
            rows = pl.ds(pl.multiple_of(a * Q, Q), Q)
            nrows = pl.ds(pl.multiple_of(jnp.minimum(a + 1, NB - 1) * Q, Q), Q)
            dh = dh_s[rows, :]
            nxt = jnp.where(a + 1 < NB, dh_s[nrows, :], jnp.zeros((Q, D), bf16))
            dw_s[a] = _dot2(gmth[...], gmtl[...], jnp.concatenate([dh, nxt], 0))
            xn = xn_s[rows, :]
            uf_s[a] = _dot2(fmh[...], fml[...], xn)
            return acc + jnp.sum(dh.astype(f32) * xn.astype(f32), axis=0, keepdims=True)
        ddsk_ref[...] = jax.lax.fori_loop(0, NB, q1, jnp.zeros((1, D), f32)).astype(bf16)

        def corr(b, other):
            def inner(a, acc):
                dw = dw_s[a]
                o = other[a - b]
                return (acc[0] + dw[:Q] * o[:Q] + dw[Q:] * o[Q:],
                        acc[1] + dw[Q:] * o[:Q] - dw[:Q] * o[Q:])
            z0 = jnp.zeros((Q, D), f32)
            r, i = jax.lax.fori_loop(b, NB, inner, (z0, z0))
            return jnp.concatenate([r, i], 0)

        def q2(b, c):
            rows = pl.ds(pl.multiple_of(b * Q, Q), Q)
            dxn = _dot3(fmth[...], fmtl[...], corr(b, kf_s))
            dh = dh_s[rows, :].astype(f32)
            xh, r = _ln(x_ref[rows, :].astype(f32))
            dx_ref[rows, :] = (dh + _ln_bwd(dxn + dh * dsk, xh, r)).astype(bf16)
            return c
        jax.lax.fori_loop(0, NB, q2, 0)

        for j in range(NB):
            ku_s[_OFFS[j]:_OFFS[j] + Q, :] += _dot3(fsth[j], fstl[j], corr(j, uf_s))
    pl.run_scoped(bwd_a, pltpu.VMEM((NB, 2 * Q, D), f32), pltpu.VMEM((NB, 2 * Q, D), f32))

    def kbwd(n, ddt):
        br, bi, cr, ci = cb_row(n)
        s0r = s0i = s1r = s1i = jnp.zeros((1, D), f32)
        for seg in SEGS:
            _, _, nk, ro = seg
            er, ei, gr, gi = seg_tables(seg, n)
            t = ku_s[ro:ro + 8 * nk, :]
            tl = (t * lcol_ref[ro:ro + 8 * nk, :]).reshape(nk, 8, D)
            t = t.reshape(nk, 8, D)
            a0r, a0i = _cmul(jnp.sum(t * gr, 0), jnp.sum(t * gi, 0), er, ei)
            a1r, a1i = _cmul(jnp.sum(tl * gr, 0), jnp.sum(tl * gi, 0), er, ei)
            s0r = s0r + jnp.sum(a0r, 0, keepdims=True)
            s0i = s0i + jnp.sum(a0i, 0, keepdims=True)
            s1r = s1r + jnp.sum(a1r, 0, keepdims=True)
            s1i = s1i + jnp.sum(a1i, 0, keepdims=True)
        row = pl.ds(n, 1)
        tr, ti = _cmul(br, bi, s0r, s0i)
        dcre_ref[row, :] = tr
        dcim_ref[row, :] = (-ti)
        tr, ti = _cmul(cr, ci, s0r, s0i)
        dbre_ref[row, :] = (dt * tr)
        dbim_ref[row, :] = (-dt * ti)
        b0r = bre_ref[row, :].astype(f32)
        b0i = bim_ref[row, :].astype(f32)
        wr, wi = _cmul(cr, ci, br, bi)
        gre, gim = _cmul(wr, wi, s1r, s1i)
        gim = -gim
        dare_ref[row, :] = (dt * gre)
        daim_ref[row, :] = (dt * gim)
        return (ddt + are_ref[row, :].astype(f32) * gre + aim_ref[row, :].astype(f32) * gim
                + tr * b0r - ti * b0i)

    def sc_bwd(pa, pb):
        fill_tables(pa, pb)
        ddt = jax.lax.fori_loop(0, N, kbwd, jnp.zeros((1, D), f32))
        dldt_ref[...] = (ddt * dt).astype(bf16)
    pl.run_scoped(sc_bwd, pltpu.VMEM((12, N, D), f32), pltpu.VMEM((12, N, D), f32))


@jax.jit
def pallas_sequential_preLN__ssm_conv_s4__mixer_gmlp__prompt_kernel(
    A_u, A_A_re, A_A_im, A_B_re, A_B_im, A_C_re, A_C_im, A_log_dt, A_Dskip,
    B_x, B_w_in, B_w_sp, B_b_sp, B_w_out, grad_out,
):
    vm = pl.BlockSpec(memory_space=pltpu.VMEM)
    hbm = pl.BlockSpec(memory_space=pl.ANY)
    sd = lambda *s: jax.ShapeDtypeStruct(s, bf16)
    ins = [A_u.reshape(S, D), grad_out.reshape(S, D), A_A_re.T.astype(f32), A_A_im.T.astype(f32), A_B_re.T.astype(f32), A_B_im.T.astype(f32),
           A_C_re.T.astype(f32), A_C_im.T.astype(f32), A_log_dt.reshape(1, D), A_Dskip.reshape(1, D), B_w_in, B_w_sp,
           B_b_sp.reshape(S, 1), B_w_out, jnp.asarray(_LCOL)]
    ins += [jnp.asarray(m) for m in _CM]
    outs = pl.pallas_call(
        _kernel,
        out_shape=[sd(S, D), sd(S, D)] + [jax.ShapeDtypeStruct((N, D), f32)] * 6 + [sd(1, D), sd(1, D), sd(D, F),
                                                            sd(S, S), sd(S, 1), sd(FH, D)],
        in_specs=[vm] * len(ins),
        out_specs=[vm] * 10 + [hbm, hbm, vm, vm],
        scratch_shapes=[pltpu.VMEM((S, D), bf16), pltpu.VMEM((S, D), bf16),
                        pltpu.VMEM((S, D), bf16), pltpu.VMEM((NB, 2 * Q, D), f32),
                        pltpu.VMEM((KU, D), f32), pltpu.SemaphoreType.DMA((2,))],
        compiler_params=pltpu.CompilerParams(vmem_limit_bytes=127 * 1024 * 1024),
    )(*ins)
    (h2, dx, dare, daim, dbre, dbim, dcre, dcim, dldt, ddsk, dwin, dwsp, dbsp, dwout) = outs
    return (h2.reshape(1, S, D), dx.reshape(1, S, D), *[t.T.astype(bf16) for t in (dare, daim, dbre, dbim, dcre, dcim)],
            dldt.reshape(D), ddsk.reshape(D), dwin, dwsp, dbsp.reshape(S), dwout)
```
